```python
import os as _os
_os.environ.setdefault("JAX_PLATFORMS", "cpu")
import jax
import jax.numpy as jnp

def _softmax(x, axis=-1):
    return jax.nn.softmax(x, axis=axis)
def _gelu(x):
    return jax.nn.gelu(x, approximate=True)
def _silu(x):
    return jax.nn.silu(x)
def _sigmoid(x):
    return jax.nn.sigmoid(x)
def _layernorm(x, axis=-1, eps=1e-5):
    m = jnp.mean(x, axis=axis, keepdims=True)
    v = jnp.var(x, axis=axis, keepdims=True)
    return (x - m) / jnp.sqrt(v + eps)
def _scatter_add(tgt, idx, src, axis=0):
    return tgt.at[idx].add(src)
def _segment_sum(src, seg, n):
    return jax.ops.segment_sum(src, seg, n)
class _Rng:
    def __init__(self, key):
        self._k = key
    def _next(self):
        self._k, sub = jax.random.split(self._k)
        return sub
    def normal(self, shape):
        return jax.random.normal(self._next(), shape, dtype=jnp.bfloat16)
    def randint(self, lo, hi, shape):
        return jax.random.randint(self._next(), shape, lo, hi, dtype=jnp.int32)
    def uniform(self, shape, lo=0.0, hi=1.0):
        return jax.random.uniform(self._next(), shape, jnp.bfloat16, lo, hi)
    def permutation(self, n):
        return jax.random.permutation(self._next(), n)


kernel_name = 'interleave_layers__sliding_block__dense_activation_gelu__prompt'

def setup_inputs():
    _rng = _Rng(jax.random.key(int.from_bytes(__import__("os").urandom(4), "little")))
    _w = (lambda a: (lambda t: t.astype(jnp.bfloat16) if jnp.issubdtype(t.dtype, jnp.floating) else t)(jnp.asarray(a)))
    def _A_setup():
        B, S, D = 1, 2048, 640
        return {
            "x": _w((lambda *s: _rng.normal(s) * 0.05)(B, S, D)),
            "wqkv": _w((lambda *s: _rng.normal(s) * 0.05)(D, 3 * D)),
            "wo": _w((lambda *s: _rng.normal(s) * 0.05)(D, D)),
        }
    _A_in = _A_setup()

    def _B_setup():
        B, S, D, F = 1, 2048, 640, 1728
        return {
            "x": _w((lambda *s: _rng.normal(s) * 0.05)(B, S, D)),
            "w1": _w((lambda *s: _rng.normal(s) * 0.8)(D, F) * (D ** -0.5)),
            "b1": _w((lambda *s: _rng.normal(s) * 0.8)(F) * 0.01),
            "w2": _w((lambda *s: _rng.normal(s) * 0.8)(F, D) * (F ** -0.5)),
            "b2": _w((lambda *s: _rng.normal(s) * 0.8)(D) * 0.01),
        }
    _B_in = _B_setup()

    return {
        "A_x": _A_in["x"],
        "A_wqkv": _A_in["wqkv"],
        "A_wo": _A_in["wo"],
        "B_x": _B_in["x"],
        "B_w1": _B_in["w1"],
        "B_b1": _B_in["b1"],
        "B_w2": _B_in["w2"],
        "B_b2": _B_in["b2"],
    }

def reference(A_x, A_wqkv, A_wo, B_x, B_w1, B_b1, B_w2, B_b2):
    def _A_ref(x, wqkv, wo):
        B, S, D = x.shape
        H = 32; Dh = D // H; W = 256
        qkv = (lambda x, *d: x.transpose(*d))((x @ wqkv).reshape(B, S, 3, H, Dh), 2, 0, 3, 1, 4)
        q, k, v = qkv[0], qkv[1], qkv[2]
        scores = jnp.einsum("bhqd,bhkd->bhqk", q, k) * (Dh ** -0.5)
        idx = jnp.arange(S)
        mask = (idx[:, None] - idx[None, :] >= 0) & (idx[:, None] - idx[None, :] < W)
        scores = jnp.where(mask[None, None], scores, -1e9)
        p = _softmax(scores, axis=-1)
        o = jnp.einsum("bhqk,bhkd->bhqd", p, v)
        return (lambda x, *d: x.transpose(*d))(o, 0, 2, 1, 3).reshape(B, S, D) @ wo

    def _B_ref(x, w1, b1, w2, b2):
        h = jnp.einsum("bsd,df->bsf", x, w1) + b1
        h = _gelu(h)
        return jnp.einsum("bsf,fd->bsd", h, w2) + b2

    x = A_x
    x = x + _A_ref(_layernorm(x, axis=-1), A_wqkv, A_wo)
    x = x + _B_ref(_layernorm(x, axis=-1), B_w1, B_b1, B_w2, B_b2)
    x = x + _A_ref(_layernorm(x, axis=-1), A_wqkv, A_wo)
    x = x + _B_ref(_layernorm(x, axis=-1), B_w1, B_b1, B_w2, B_b2)
    return x
```

```python
import functools
import numpy as np
import jax
import jax.numpy as jnp
from jax import lax
import jax.experimental.pallas as pl
import jax.experimental.pallas.tpu as pltpu

S, D, H, DH, W, F = 2048, 640, 32, 20, 256, 1728
QB = 128
KW = W + QB
KW2 = W + 64
NT = (((1,), (1,)), ((), ()))
TN = (((0,), (0,)), ((), ()))
bf16, f32 = jnp.bfloat16, jnp.float32
LOG2E = 1.4426950408889634


def _ln(x):
    m = jnp.mean(x, axis=-1, keepdims=True)
    xc = x - m
    v = jnp.mean(xc * xc, axis=-1, keepdims=True)
    return xc * lax.rsqrt(v + 1e-5)


def _gelu(h):
    c = 0.7978845608028654
    return 0.5 * h * (1.0 + jnp.tanh(c * (h + 0.044715 * (h * h * h))))


def _shift64(t):
    return t[:, 64:64 + 512]


def make_kernel(TM, ATT=True, FFN=True, NH=H, ORD=0, UNR=1, NC1=1, NC2=1):
    NQ = TM // QB

    def kernel(x_ref, wqkv_ref, wo_hbm, w1_hbm, b1_ref, w2_hbm, b2_ref, o_ref,
               wo_ref, w1_ref, w2_ref, sems,
               wvt_s, k_s, vt_s, q_s, ot_s, bias_s, x_s, sa_s, sb_s, ma_s, mb_s):
        step = pl.program_id(0)

        copies = [pltpu.make_async_copy(wo_hbm, wo_ref, sems.at[0]),
                  pltpu.make_async_copy(w1_hbm, w1_ref, sems.at[1]),
                  pltpu.make_async_copy(w2_hbm, w2_ref, sems.at[2])]

        @pl.when(step == 0)
        def _():
            for cp in copies:
                cp.start()
            wvt_s[...] = wqkv_ref[:, 2 * D:].astype(f32).T.astype(bf16)
            r = lax.broadcasted_iota(jnp.int32, (64, QB), 0)
            c = lax.broadcasted_iota(jnp.int32, (64, QB), 1) & 63
            bias_s[0] = jnp.where(r > c, 0.0, -1e9).astype(f32)
            bias_s[1] = jnp.where(r <= c, 0.0, -1e9).astype(f32)
            k_s[:, :W // 2, :] = jnp.zeros((18, W // 2, 128), jnp.int32)
            vt_s[:, :, :W] = jnp.zeros((2, D // 2, W), jnp.int32)

        x_s[...] = x_ref[...].astype(f32)
        row0 = pl.multiple_of(step * TM, TM)

        def layer(l, carry):
            hrow0 = pl.multiple_of((W + row0) // 2, TM // 2 if TM <= W else W // 2)
            C1 = TM // NC1
            for c in range(NC1):
                xn = _ln(x_s[c * C1:(c + 1) * C1]).astype(bf16)
                qk = jnp.dot(xn, wqkv_ref[:, :2 * D], preferred_element_type=f32)
                q = qk[:, :D] * (DH ** -0.5 * LOG2E)
                k = qk[:, D:]
                qsh = _shift64(q).astype(bf16)
                ksh = _shift64(k).astype(bf16)
                q = q.astype(bf16)
                k = k.astype(bf16)
                for w in range(9):
                    src_q, src_k, c0 = (q, k, w * 128) if w < 5 else (qsh, ksh, (w - 5) * 128)
                    q_s[w, c * C1 // 2:(c + 1) * C1 // 2] = pltpu.bitcast(src_q[:, c0:c0 + 128], jnp.int32)
                    k_s[l * 9 + w, pl.ds(hrow0 + c * C1 // 2, C1 // 2), :] = pltpu.bitcast(
                        src_k[:, c0:c0 + 128], jnp.int32)
                vt = lax.dot_general(wvt_s[...], xn, NT, preferred_element_type=f32)
                vt_s[l, :, pl.ds(W + row0 + c * C1, C1)] = pltpu.bitcast(vt.astype(bf16), jnp.int32)

            lane = lax.broadcasted_iota(jnp.int32, (1, 128), 1)
            rowi = lax.broadcasted_iota(jnp.int32, (16, 128), 0)

            def pens(i, u):
                hb = 2 * i + u
                return [jnp.where(hb + b >= 4, 0.0, -1e9).astype(f32) for b in range(4)]

            def phase1(t, s_buf, m_buf):
                j = t >> 3
                g = t & 7
                i = step * NQ + j
                for r in range(4):
                    u = r & 1
                    lo = 2 * DH * (2 * g + (r >> 1))
                    ins = (lo & 127) + 2 * DH <= 128
                    w = jnp.where(ins, lo >> 7, 5 + ((lo - 64) >> 7))
                    off = jnp.where(ins, lo & 127, (lo - 64) & 127)
                    qh = q_s[w, pl.ds(pl.multiple_of(j * 64 + 32 * u, 32), 32), :]
                    qa = jnp.where((lane >= off) & (lane < off + DH), qh, 0)
                    qb = jnp.where((lane >= off + DH) & (lane < off + 2 * DH), qh, 0)
                    qbd = pltpu.bitcast(jnp.concatenate([qb, qa] if u else [qa, qb], axis=0), bf16)
                    kh = pltpu.bitcast(
                        k_s[l * 9 + w, pl.ds(pl.multiple_of(i * 64 + 32 * u, 32), KW2 // 2), :], bf16)
                    sc = lax.dot_general(kh, qbd, NT, preferred_element_type=f32)
                    pn = pens(i, u)
                    blk = [sc[:64] + bias_s[0], sc[64:128], sc[128:192], sc[192:256], sc[256:] + bias_s[1]]
                    m8 = None
                    for b in range(5):
                        s_buf[r, 64 * b:64 * (b + 1)] = blk[b]
                        mb = jnp.max(blk[b].reshape(8, 8, 128), axis=0)
                        if b < 4:
                            mb = mb + pn[b]
                        m8 = mb if m8 is None else jnp.maximum(m8, mb)
                    m = jnp.max(m8, axis=0, keepdims=True)
                    m_buf[r] = jnp.broadcast_to(m, (8, 128))

            def phase2(t, s_buf, m_buf):
                j = t >> 3
                g = t & 7
                i = step * NQ + j
                krow = pl.multiple_of(i * QB, QB)
                qrow = pl.multiple_of(j * QB, QB)
                outs = []
                for r in range(4):
                    u = r & 1
                    odd = r >> 1
                    m = m_buf[r][:1]
                    pn = pens(i, u)
                    ps = [jnp.exp2(s_buf[r, 64 * b:64 * (b + 1)] - ((m - pn[b]) if b < 4 else m))
                          for b in range(5)]
                    z = [jnp.zeros((64, 128), f32)]
                    p = jnp.concatenate(z + ps if u else ps + z, axis=0).astype(bf16)
                    v0 = pl.multiple_of(40 * g + 16 * odd, 8)
                    one_row = 0 if odd else 40
                    vh = vt_s[l, pl.ds(v0, 24), pl.ds(krow, KW)]
                    ri = lax.broadcasted_iota(jnp.int32, (24, KW), 0)
                    vh = jnp.where(ri == one_row // 2, (vh & (0xFFFF0000 - (1 << 32))) | 0x3F80, vh)
                    o = jnp.dot(pltpu.bitcast(vh, bf16), p, preferred_element_type=f32)
                    outs.append(o * (1.0 / o[one_row:one_row + 1, :]))
                low = lax.broadcasted_iota(jnp.int32, (8, 128), 1) < 64
                rr = lax.broadcasted_iota(jnp.int32, (8, 128), 0)
                pieces = []
                for odd in range(2):
                    u0, u1 = outs[2 * odd], outs[2 * odd + 1]
                    for v in range(odd, 5 + odd):
                        a0, a1 = u0[8 * v:8 * v + 8], u1[8 * v:8 * v + 8]
                        last_a = 20 + 8 * odd - 8 * v
                        if last_a >= 8:
                            pieces.append(jnp.where(low, a0, a1))
                        elif last_a <= 0:
                            pieces.append(pltpu.roll(jnp.where(low, a1, a0), 64, 1))
                        else:
                            pieces.append(jnp.where(rr < last_a, jnp.where(low, a0, a1),
                                                    pltpu.roll(jnp.where(low, a1, a0), 64, 1)))
                ot_s[pl.ds(pl.multiple_of(80 * g, 16), 80), pl.ds(qrow, QB)] = (
                    jnp.concatenate(pieces, axis=0).astype(bf16))

            NS = NQ * 8
            if ATT:
                phase1(0, sa_s, ma_s)

                def pair(u, c):
                    t = 2 * u
                    if ORD == 0:
                        phase1(t + 1, sb_s, mb_s)
                        phase2(t, sa_s, ma_s)
                        phase1(jnp.minimum(t + 2, NS - 1), sa_s, ma_s)
                        phase2(t + 1, sb_s, mb_s)
                    else:
                        phase2(t, sa_s, ma_s)
                        phase1(t + 1, sb_s, mb_s)
                        phase2(t + 1, sb_s, mb_s)
                        phase1(jnp.minimum(t + 2, NS - 1), sa_s, ma_s)
                    return c

                lax.fori_loop(0, NS // 2, pair, 0, unroll=UNR)
            @pl.when((step == 0) & (l == 0))
            def _():
                for cp in copies:
                    cp.wait()

            C2 = TM // NC2
            for c in range(NC2):
                rs = slice(c * C2, (c + 1) * C2)
                y = lax.dot_general(ot_s[:, rs], wo_ref[...], TN, preferred_element_type=f32)
                x = x_s[rs] + y
                xn = _ln(x).astype(bf16)
                hh = lax.dot_general(xn, w1_ref[...], NT, preferred_element_type=f32) + b1_ref[...].astype(f32).reshape(1, F)
                g = _gelu(hh).astype(bf16)
                y = jnp.dot(g, w2_ref[...], preferred_element_type=f32) + b2_ref[...].astype(f32).reshape(1, D)
                x_s[rs] = x + y
            return carry

        lax.fori_loop(0, 2, layer, 0)
        o_ref[...] = x_s[...].astype(o_ref.dtype)

    return kernel


def build(TM=256, **kw):
    def fn(A_x, A_wqkv, A_wo, B_x, B_w1, B_b1, B_w2, B_b2):
        x2 = A_x.reshape(S, D)
        full = lambda shp: pl.BlockSpec(shp, lambda i: (0,) * len(shp))
        hbm = pl.BlockSpec(memory_space=pl.ANY)
        out = pl.pallas_call(
            make_kernel(TM, **kw),
            grid=(S // TM,),
            in_specs=[pl.BlockSpec((TM, D), lambda i: (i, 0)), full((D, 3 * D)), hbm, hbm,
                      full((F,)), hbm, full((D,))],
            out_specs=pl.BlockSpec((TM, D), lambda i: (i, 0)),
            out_shape=jax.ShapeDtypeStruct((S, D), A_x.dtype),
            scratch_shapes=[
                pltpu.VMEM((D, D), bf16), pltpu.VMEM((F, D), bf16), pltpu.VMEM((F, D), bf16),
                pltpu.SemaphoreType.DMA((3,)),
                pltpu.VMEM((D, D), bf16),
                pltpu.VMEM((18, (S + W) // 2, 128), jnp.int32),
                pltpu.VMEM((2, D // 2, S + W), jnp.int32),
                pltpu.VMEM((9, TM // 2, 128), jnp.int32),
                pltpu.VMEM((D, TM), bf16),
                pltpu.VMEM((2, 64, QB), f32),
                pltpu.VMEM((TM, D), f32),
                pltpu.VMEM((4, KW2, QB), f32),
                pltpu.VMEM((4, KW2, QB), f32),
                pltpu.VMEM((4, 8, QB), f32),
                pltpu.VMEM((4, 8, QB), f32),
            ],
            compiler_params=pltpu.CompilerParams(
                dimension_semantics=("arbitrary",), vmem_limit_bytes=100 * 1024 * 1024),
        )(x2, A_wqkv, A_wo, B_w1.T, B_b1, B_w2, B_b2)
        return out.reshape(A_x.shape)
    return fn


@jax.jit
def pallas_interleave_layers__sliding_block__dense_activation_gelu__prompt_kernel(
    A_x, A_wqkv, A_wo, B_x, B_w1, B_b1, B_w2, B_b2):
    return build(TM=512,UNR=8,NC1=2)(A_x, A_wqkv, A_wo, B_x, B_w1, B_b1, B_w2, B_b2)
```

```python
import functools
import numpy as np
import jax
import jax.numpy as jnp
from jax import lax
import jax.experimental.pallas as pl
import jax.experimental.pallas.tpu as pltpu

S, D, H, DH, W, F = 2048, 640, 32, 20, 256, 1728
QB = 128
KW = W + QB
KW2 = W + 64
NT = (((1,), (1,)), ((), ()))
TN = (((0,), (0,)), ((), ()))
bf16, f32 = jnp.bfloat16, jnp.float32
LOG2E = 1.4426950408889634


def _ln(x):
    m = jnp.mean(x, axis=-1, keepdims=True)
    xc = x - m
    v = jnp.mean(xc * xc, axis=-1, keepdims=True)
    return xc * lax.rsqrt(v + 1e-5)


def _gelu(h):
    c = 0.7978845608028654
    return 0.5 * h * (1.0 + jnp.tanh(c * (h + 0.044715 * (h * h * h))))


def _shift64(t):
    return t[:, 64:64 + 512]


def make_kernel(TM, ATT=True, FFN=True, NH=H, ORD=0, UNR=1, NC1=1, NC2=1):
    NQ = TM // QB

    def kernel(x_ref, wqkv_ref, wo_hbm, w1_hbm, b1_ref, w2_hbm, b2_ref, o_ref,
               wo_ref, w1_ref, w2_ref, sems,
               wvt_s, k_s, vt_s, q_s, ot_s, bias_s, x_s, sa_s, sb_s, ma_s, mb_s):
        step = pl.program_id(0)

        copies = [pltpu.make_async_copy(wo_hbm, wo_ref, sems.at[0]),
                  pltpu.make_async_copy(w1_hbm, w1_ref, sems.at[1]),
                  pltpu.make_async_copy(w2_hbm, w2_ref, sems.at[2])]

        @pl.when(step == 0)
        def _():
            for cp in copies:
                cp.start()
            wvt_s[...] = wqkv_ref[:, 2 * D:].astype(f32).T.astype(bf16)
            r = lax.broadcasted_iota(jnp.int32, (64, QB), 0)
            c = lax.broadcasted_iota(jnp.int32, (64, QB), 1) & 63
            bias_s[0] = jnp.where(r > c, 0.0, -1e9).astype(f32)
            bias_s[1] = jnp.where(r <= c, 0.0, -1e9).astype(f32)
            k_s[:, :W // 2, :] = jnp.zeros((18, W // 2, 128), jnp.int32)
            vt_s[:, :, :W] = jnp.zeros((2, D // 2, W), jnp.int32)

        x_s[...] = x_ref[...].astype(f32)
        row0 = pl.multiple_of(step * TM, TM)

        def layer(l, carry):
            hrow0 = pl.multiple_of((W + row0) // 2, TM // 2 if TM <= W else W // 2)
            C1 = TM // NC1
            for c in range(NC1):
                xn = _ln(x_s[c * C1:(c + 1) * C1]).astype(bf16)
                qk = jnp.dot(xn, wqkv_ref[:, :2 * D], preferred_element_type=f32)
                q = qk[:, :D] * (DH ** -0.5 * LOG2E)
                k = qk[:, D:]
                qsh = _shift64(q).astype(bf16)
                ksh = _shift64(k).astype(bf16)
                q = q.astype(bf16)
                k = k.astype(bf16)
                for w in range(9):
                    src_q, src_k, c0 = (q, k, w * 128) if w < 5 else (qsh, ksh, (w - 5) * 128)
                    q_s[w, c * C1 // 2:(c + 1) * C1 // 2] = pltpu.bitcast(src_q[:, c0:c0 + 128], jnp.int32)
                    k_s[l * 9 + w, pl.ds(hrow0 + c * C1 // 2, C1 // 2), :] = pltpu.bitcast(
                        src_k[:, c0:c0 + 128], jnp.int32)
                vt = lax.dot_general(wvt_s[...], xn, NT, preferred_element_type=f32)
                vt_s[l, :, pl.ds(W + row0 + c * C1, C1)] = pltpu.bitcast(vt.astype(bf16), jnp.int32)

            @pl.when((step == 0) & (l == 0))
            def _():
                for cp in copies:
                    cp.wait()

            lane = lax.broadcasted_iota(jnp.int32, (1, 128), 1)
            rowi = lax.broadcasted_iota(jnp.int32, (16, 128), 0)

            def pens(i, u):
                hb = 2 * i + u
                return [jnp.where(hb + b >= 4, 0.0, -1e9).astype(f32) for b in range(4)]

            def phase1(t, s_buf, m_buf):
                j = t >> 3
                g = t & 7
                i = step * NQ + j
                for r in range(4):
                    u = r & 1
                    lo = 2 * DH * (2 * g + (r >> 1))
                    ins = (lo & 127) + 2 * DH <= 128
                    w = lo >> 7 if ins else 5 + ((lo - 64) >> 7)
                    off = lo & 127 if ins else (lo - 64) & 127
                    qh = q_s[w, pl.ds(j * 64 + 32 * u, 32), :]
                    qa = jnp.where((lane >= off) & (lane < off + DH), qh, 0)
                    qb = jnp.where((lane >= off + DH) & (lane < off + 2 * DH), qh, 0)
                    qbd = pltpu.bitcast(jnp.concatenate([qb, qa] if u else [qa, qb], axis=0), bf16)
                    kh = pltpu.bitcast(
                        k_s[l * 9 + w, pl.ds(pl.multiple_of(i * 64 + 32 * u, 32), KW2 // 2), :], bf16)
                    sc = lax.dot_general(kh, qbd, NT, preferred_element_type=f32)
                    pn = pens(i, u)
                    blk = [sc[:64] + bias_s[0], sc[64:128], sc[128:192], sc[192:256], sc[256:] + bias_s[1]]
                    m8 = None
                    for b in range(5):
                        s_buf[r, 64 * b:64 * (b + 1)] = blk[b]
                        mb = jnp.max(blk[b].reshape(8, 8, 128), axis=0)
                        if b < 4:
                            mb = mb + pn[b]
                        m8 = mb if m8 is None else jnp.maximum(m8, mb)
                    m = jnp.max(m8, axis=0, keepdims=True)
                    m_buf[r] = jnp.broadcast_to(m, (8, 128))

            def phase2(t, s_buf, m_buf):
                j = t >> 3
                g = t & 7
                i = step * NQ + j
                krow = pl.multiple_of(i * QB, QB)
                qrow = j * QB
                outs = []
                for r in range(4):
                    u = r & 1
                    odd = r >> 1
                    m = m_buf[r][:1]
                    pn = pens(i, u)
                    ps = [jnp.exp2(s_buf[r, 64 * b:64 * (b + 1)] - ((m - pn[b]) if b < 4 else m))
                          for b in range(5)]
                    z = [jnp.zeros((64, 128), f32)]
                    p = jnp.concatenate(z + ps if u else ps + z, axis=0).astype(bf16)
                    v0 = 40 * g + 16 * odd
                    one_row = 0 if odd else 40
                    vh = vt_s[l, pl.ds(v0, 24), pl.ds(krow, KW)]
                    ri = lax.broadcasted_iota(jnp.int32, (24, KW), 0)
                    vh = jnp.where(ri == one_row // 2, (vh & (0xFFFF0000 - (1 << 32))) | 0x3F80, vh)
                    o = jnp.dot(pltpu.bitcast(vh, bf16), p, preferred_element_type=f32)
                    outs.append(o * (1.0 / o[one_row:one_row + 1, :]))
                low = lax.broadcasted_iota(jnp.int32, (8, 128), 1) < 64
                rr = lax.broadcasted_iota(jnp.int32, (8, 128), 0)
                pieces = []
                for odd in range(2):
                    u0, u1 = outs[2 * odd], outs[2 * odd + 1]
                    for v in range(odd, 5 + odd):
                        a0, a1 = u0[8 * v:8 * v + 8], u1[8 * v:8 * v + 8]
                        last_a = 20 + 8 * odd - 8 * v
                        if last_a >= 8:
                            pieces.append(jnp.where(low, a0, a1))
                        elif last_a <= 0:
                            pieces.append(pltpu.roll(jnp.where(low, a1, a0), 64, 1))
                        else:
                            pieces.append(jnp.where(rr < last_a, jnp.where(low, a0, a1),
                                                    pltpu.roll(jnp.where(low, a1, a0), 64, 1)))
                ot_s[pl.ds(80 * g, 80), pl.ds(qrow, QB)] = (
                    jnp.concatenate(pieces, axis=0).astype(bf16))

            NS = NQ * 8
            bufs = [(sa_s, ma_s), (sb_s, mb_s)]
            phase1(0, *bufs[0])
            for t in range(NS):
                if t + 1 < NS:
                    phase1(t + 1, *bufs[(t + 1) & 1])
                phase2(t, *bufs[t & 1])

            C2 = TM // NC2
            for c in range(NC2):
                rs = slice(c * C2, (c + 1) * C2)
                y = lax.dot_general(ot_s[:, rs], wo_ref[...], TN, preferred_element_type=f32)
                x = x_s[rs] + y
                xn = _ln(x).astype(bf16)
                hh = lax.dot_general(xn, w1_ref[...], NT, preferred_element_type=f32) + b1_ref[...].astype(f32).reshape(1, F)
                g = _gelu(hh).astype(bf16)
                y = jnp.dot(g, w2_ref[...], preferred_element_type=f32) + b2_ref[...].astype(f32).reshape(1, D)
                x_s[rs] = x + y
            return carry

        lax.fori_loop(0, 2, layer, 0)
        o_ref[...] = x_s[...].astype(o_ref.dtype)

    return kernel


def build(TM=256, FLAGS=None, **kw):
    def fn(A_x, A_wqkv, A_wo, B_x, B_w1, B_b1, B_w2, B_b2):
        x2 = A_x.reshape(S, D)
        full = lambda shp: pl.BlockSpec(shp, lambda i: (0,) * len(shp))
        hbm = pl.BlockSpec(memory_space=pl.ANY)
        out = pl.pallas_call(
            make_kernel(TM, **kw),
            grid=(S // TM,),
            in_specs=[pl.BlockSpec((TM, D), lambda i: (i, 0)), full((D, 3 * D)), hbm, hbm,
                      full((F,)), hbm, full((D,))],
            out_specs=pl.BlockSpec((TM, D), lambda i: (i, 0)),
            out_shape=jax.ShapeDtypeStruct((S, D), A_x.dtype),
            scratch_shapes=[
                pltpu.VMEM((D, D), bf16), pltpu.VMEM((F, D), bf16), pltpu.VMEM((F, D), bf16),
                pltpu.SemaphoreType.DMA((3,)),
                pltpu.VMEM((D, D), bf16),
                pltpu.VMEM((18, (S + W) // 2, 128), jnp.int32),
                pltpu.VMEM((2, D // 2, S + W), jnp.int32),
                pltpu.VMEM((9, TM // 2, 128), jnp.int32),
                pltpu.VMEM((D, TM), bf16),
                pltpu.VMEM((2, 64, QB), f32),
                pltpu.VMEM((TM, D), f32),
                pltpu.VMEM((4, KW2, QB), f32),
                pltpu.VMEM((4, KW2, QB), f32),
                pltpu.VMEM((4, 8, QB), f32),
                pltpu.VMEM((4, 8, QB), f32),
            ],
            compiler_params=pltpu.CompilerParams(
                dimension_semantics=("arbitrary",), vmem_limit_bytes=100 * 1024 * 1024, flags=FLAGS),
        )(x2, A_wqkv, A_wo, B_w1.T, B_b1, B_w2, B_b2)
        return out.reshape(A_x.shape)
    return fn


@jax.jit
def pallas_interleave_layers__sliding_block__dense_activation_gelu__prompt_kernel(
    A_x, A_wqkv, A_wo, B_x, B_w1, B_b1, B_w2, B_b2):
    return build(TM=512,NC1=2)(A_x, A_wqkv, A_wo, B_x, B_w1, B_b1, B_w2, B_b2)
```
